```python
import jax
import jax.numpy as jnp

def _softmax(x, axis=-1):
    return jax.nn.softmax(x, axis=axis)
def _gelu(x):
    return jax.nn.gelu(x, approximate=True)
def _silu(x):
    return jax.nn.silu(x)
def _sigmoid(x):
    return jax.nn.sigmoid(x)
def _layernorm(x, axis=-1, eps=1e-5):
    m = jnp.mean(x, axis=axis, keepdims=True)
    v = jnp.var(x, axis=axis, keepdims=True)
    return (x - m) / jnp.sqrt(v + eps)
def _scatter_add(tgt, idx, src, axis=0):
    return tgt.at[idx].add(src)
def _segment_sum(src, seg, n):
    return jax.ops.segment_sum(src, seg, n)
class _Rng:
    def __init__(self, key):
        self._k = key
    def _next(self):
        self._k, sub = jax.random.split(self._k)
        return sub
    def normal(self, shape):
        return jax.random.normal(self._next(), shape, dtype=jnp.bfloat16)
    def randint(self, lo, hi, shape):
        return jax.random.randint(self._next(), shape, lo, hi, dtype=jnp.int32)
    def uniform(self, shape, lo=0.0, hi=1.0):
        return jax.random.uniform(self._next(), shape, jnp.bfloat16, lo, hi)
    def permutation(self, n):
        return jax.random.permutation(self._next(), n)


kernel_name = 'standalone__groupnorm__prompt'

def setup_inputs():
    _rng = _Rng(jax.random.key(int.from_bytes(__import__("os").urandom(4), "little")))
    _w = (lambda a: (lambda t: t.astype(jnp.bfloat16) if jnp.issubdtype(t.dtype, jnp.floating) else t)(jnp.asarray(a)))
    B = 2
    G = 32
    cpg = max(1, 1024 // G)
    C = G * cpg
    H, W = 32, 2048
    return {
        "x": _w((lambda *s: _rng.normal(s) * 0.05)(B, C, H, W)),
        "g": _w((lambda *s: _rng.normal(s) * 0.05)(C) + 1.0),
        "b": _w((lambda *s: _rng.normal(s) * 0.05)(C)),
    }

def reference(x, g, b):
    G = 32
    B, C, H, W = x.shape[0], x.shape[1], x.shape[2], x.shape[3]
    xr = x.reshape(B, G, C // G, H, W)
    mu = xr.mean(axis=(2, 3, 4), keepdims=True)
    var = ((xr - mu) ** 2).mean(axis=(2, 3, 4), keepdims=True)
    xn = (xr - mu) / jnp.sqrt(var + 1e-5)
    xn = xn.reshape(B, C, H, W)
    return xn * g[None, :, None, None] + b[None, :, None, None]
```

```python
import jax
import jax.numpy as jnp
from jax import lax
import jax.experimental.pallas as pl
import jax.experimental.pallas.tpu as pltpu

GROUPS = 32
EPS = 1e-5

SLAB_ROWS = 8
SLABS = 32
PHASE = 16
REGION = 2
LANE_SPLIT = 2
READ_TAIL = 8
WRITE_TAIL = 2
CH_PER_ITER = 2
ACC_LANES = 512


@jax.jit
def pallas_standalone__groupnorm__prompt_kernel(
    x: jax.Array,
    g: jax.Array,
    b: jax.Array,
):
    B, C, H, W = x.shape
    cpg = C // GROUPS
    n_groups = B * GROUPS
    spc = H // SLAB_ROWS
    rpg = cpg * spc // SLABS
    iters_per_row = SLABS // spc // CH_PER_ITER
    n_regions = PHASE // REGION
    n_phases = n_groups // PHASE
    piece = W // LANE_SPLIT
    p_rows = C // 128
    inv_n = 1.0 / (cpg * H * W)
    f32 = jnp.float32
    assert H % SLAB_ROWS == 0 and (cpg * spc) % SLABS == 0 and rpg > 1
    assert SLABS % (spc * CH_PER_ITER) == 0 and 128 % cpg == 0 and C % 128 == 0
    assert n_groups % PHASE == 0 and PHASE % REGION == 0 and n_regions >= 2

    def kernel(x_ref, g_ref, b_ref, o_ref, buf, gb_in, gb_f32, gb_smem, rsem, wsem, psem):
        def read(i, j):
            return pltpu.make_async_copy(
                x_ref.at[pl.ds(i * rpg, rpg)], buf.at[pl.ds(j * rpg, rpg)], rsem.at[j])

        def read_last(i):
            src, dst = i * rpg + rpg - 1, PHASE * rpg - 1
            head, tail = pl.ds(0, SLABS - READ_TAIL), pl.ds(SLABS - READ_TAIL, READ_TAIL)
            return (
                pltpu.make_async_copy(x_ref.at[pl.ds(i * rpg, rpg - 1)],
                                      buf.at[pl.ds((PHASE - 1) * rpg, rpg - 1)], rsem.at[PHASE - 1]),
                pltpu.make_async_copy(x_ref.at[src, head], buf.at[dst, head], rsem.at[PHASE]),
                pltpu.make_async_copy(x_ref.at[src, tail], buf.at[dst, tail], rsem.at[PHASE + 1]),
            )

        def start_other_reads(p):
            @pl.loop(1, PHASE - 1)
            def _(j):
                read(p * PHASE + j, j).start()

            for copy in read_last(p * PHASE + PHASE - 1):
                copy.start()

        def region_rows(p, r):
            n = REGION * rpg
            return pl.ds(r * n, n), pl.ds(p * PHASE * rpg + r * n, n)

        def start_writes(p, r, lo, hi, sem):
            src, dst = region_rows(p, r)

            @pl.loop(lo, hi)
            def _(s):
                for h in range(LANE_SPLIT):
                    lanes = pl.ds(h * piece, piece)
                    pltpu.make_async_copy(
                        buf.at[src, s, :, lanes], o_ref.at[dst, s, :, lanes], sem).start()

        def wait_writes(p, r, lo, hi, sem):
            src, dst = region_rows(p, r)
            cols = pl.ds(lo, hi - lo)
            pltpu.make_async_copy(buf.at[src, cols], o_ref.at[dst, cols], sem).wait()

        def fold(v):
            parts = [v[:, k:k + ACC_LANES] for k in range(0, W, ACC_LANES)]
            while len(parts) > 1:
                parts = [parts[k] + parts[k + 1] for k in range(0, len(parts), 2)]
            return parts[0]

        def mean_of(acc):
            return jnp.sum(jnp.sum(acc, axis=0, keepdims=True), axis=1, keepdims=True) * inv_n

        def normalize(i, j):
            n_iters = cpg // CH_PER_ITER
            zeros = jnp.zeros((SLAB_ROWS, ACC_LANES), f32)

            def position(t):
                return (j * rpg + lax.div(t, iters_per_row),
                        lax.rem(t, iters_per_row) * (CH_PER_ITER * spc))

            def add_values(t, acc):
                row, s = position(t)
                for k in range(CH_PER_ITER * spc):
                    acc = acc + fold(buf[row, s + k].astype(f32))
                return acc

            mu = mean_of(lax.fori_loop(0, n_iters, add_values, zeros))

            def add_squares(t, acc):
                row, s = position(t)
                for k in range(CH_PER_ITER * spc):
                    d = buf[row, s + k].astype(f32) - mu
                    acc = acc + fold(d * d)
                return acc

            var = mean_of(lax.fori_loop(0, n_iters, add_squares, zeros))
            rstd = 1.0 / jnp.sqrt(var + EPS)

            ch0 = lax.rem(i, GROUPS) * cpg
            p_row, p_col = lax.div(ch0, 128), lax.rem(ch0, 128)

            @pl.loop(0, n_iters)
            def _(t):
                row, s = position(t)
                for c in range(CH_PER_ITER):
                    col = p_col + t * CH_PER_ITER + c
                    scale = rstd * gb_smem[p_row, col]
                    shift = gb_smem[p_rows + p_row, col]
                    for k in range(c * spc, (c + 1) * spc):
                        d = buf[row, s + k].astype(f32) - mu
                        buf[row, s + k] = (d * scale + shift).astype(buf.dtype)

        g_copy = pltpu.make_async_copy(g_ref, gb_in.at[0], psem.at[0])
        b_copy = pltpu.make_async_copy(b_ref, gb_in.at[1], psem.at[1])
        read(0, 0).start()
        g_copy.start()
        b_copy.start()
        start_other_reads(0)
        g_copy.wait()
        b_copy.wait()
        gb_f32[pl.ds(0, p_rows)] = gb_in[0].astype(f32)
        gb_f32[pl.ds(p_rows, p_rows)] = gb_in[1].astype(f32)
        to_smem = pltpu.make_async_copy(gb_f32, gb_smem, psem.at[0])
        to_smem.start()
        to_smem.wait()

        last, split = n_regions - 1, SLABS - WRITE_TAIL

        @pl.loop(0, n_groups)
        def _(i):
            p, j = lax.div(i, PHASE), lax.rem(i, PHASE)

            @pl.when(j < PHASE - 1)
            def _():
                read(i, j).wait()

            @pl.when(j == PHASE - 1)
            def _():
                bulk, head, tail = read_last(i)
                bulk.wait()
                head.wait()
                start_writes(p, 0, 0, SLABS, wsem.at[0])
                tail.wait()

            normalize(i, j)

            @pl.when(j == PHASE - 1)
            def _():
                @pl.loop(1, last)
                def _(r):
                    start_writes(p, r, 0, SLABS, wsem.at[r])

                start_writes(p, last, 0, split, wsem.at[last])
                start_writes(p, last, split, SLABS, wsem.at[last + 1])

                @pl.loop(0, last)
                def _(r):
                    wait_writes(p, r, 0, SLABS, wsem.at[r])

                wait_writes(p, last, 0, split, wsem.at[last])

                @pl.when(p + 1 < n_phases)
                def _():
                    read(i + 1, 0).start()

                wait_writes(p, last, split, SLABS, wsem.at[last + 1])

                @pl.when(p + 1 < n_phases)
                def _():
                    start_other_reads(p + 1)

    view = (n_groups * rpg, SLABS, SLAB_ROWS, W)
    hbm = pl.BlockSpec(memory_space=pltpu.HBM)
    out = pl.pallas_call(
        kernel,
        in_specs=[hbm, hbm, hbm],
        out_specs=hbm,
        out_shape=jax.ShapeDtypeStruct(view, x.dtype),
        scratch_shapes=[
            pltpu.VMEM((PHASE * rpg, SLABS, SLAB_ROWS, W), x.dtype),
            pltpu.VMEM((2, p_rows, 128), g.dtype),
            pltpu.VMEM((2 * p_rows, 128), f32),
            pltpu.SMEM((2 * p_rows, 128), f32),
            pltpu.SemaphoreType.DMA((PHASE + 2,)),
            pltpu.SemaphoreType.DMA((n_regions + 1,)),
            pltpu.SemaphoreType.DMA((2,)),
        ],
        compiler_params=pltpu.CompilerParams(vmem_limit_bytes=100 * 2**20),
    )(x.reshape(view), g.reshape(p_rows, 128), b.reshape(p_rows, 128))
    return out.reshape(x.shape)
```

```python
import jax
import jax.numpy as jnp
from jax import lax
import jax.experimental.pallas as pl
import jax.experimental.pallas.tpu as pltpu

GROUPS = 32
EPS = 1e-5

SLAB_ROWS = 8
SLABS = 32
HELD = 2
PHASE = 10
PERIOD = 11
LONG_EVERY = 5
LEAD = (2, 0, 0)
READ_TAIL = 2
WRITE_TAIL = 1
BURST = 3
BURSTS_PER_ROW = 11
CH_PER_ITER = 8
ACC_LANES = 512
TASKS = 5


def _period_edges(cols, lead):
    edges = [lead]
    while edges[-1] < cols - READ_TAIL:
        j = len(edges)
        edges.append(min(lead + j * PERIOD + j // LONG_EVERY, cols - READ_TAIL))
    return edges


def _divmod(i, n):
    assert n & (n - 1) == 0
    return i >> (n.bit_length() - 1), i & (n - 1)


def _count(hi, lo, n, step):
    wrap = step & (lo == n - 1)
    return hi + wrap.astype(jnp.int32), jnp.where(wrap, 0, lo + step.astype(jnp.int32))


@jax.jit
def pallas_standalone__groupnorm__prompt_kernel(
    x: jax.Array,
    g: jax.Array,
    b: jax.Array,
):
    B, C, H, W = x.shape
    cpg = C // GROUPS
    spc = H // SLAB_ROWS
    rpg = cpg * spc // SLABS
    rpr = 2 * rpg
    cols = 2 * SLABS
    half = W // 2
    n_regions = B * GROUPS // 2
    n_phases = len(LEAD)
    burst_cols = BURST * BURSTS_PER_ROW
    n_iters = cpg // CH_PER_ITER
    per_iter = CH_PER_ITER * spc
    iters_per_row = SLABS // per_iter
    p_rows = C // 128
    inv_n = 1.0 / (cpg * H * W)
    f32 = jnp.float32
    assert H % SLAB_ROWS == 0 and (cpg * spc) % SLABS == 0 and SLABS % (spc * CH_PER_ITER) == 0
    assert 128 % cpg == 0 and C % 128 == 0 and HELD + n_phases * PHASE == n_regions
    assert 0 < cols - burst_cols <= SLABS and cols > TASKS * (PERIOD + 1)

    edges = [_period_edges((PHASE + (0 if p else HELD)) * cols, LEAD[p]) for p in range(n_phases)]
    n_periods = [len(e) - 1 for e in edges]
    period_sizes = sorted({hi - lo for e in edges for lo, hi in zip(e, e[1:])} | {READ_TAIL})
    lead_sizes = sorted(set(LEAD) - {0})

    def kernel(x_ref, g_ref, b_ref, o_ref, buf, stats, gb_in, gb_f32, gb_smem,
               read_sem, write_sem, burst_sem, param_sem):
        def half_slab(ref, rows, w):
            slab, side = _divmod(w, 2)
            return ref.at[rows, slab, :, pl.ds(pl.multiple_of(side * half, half), half)]

        def column(p, c, hbm_ref):
            region, w = _divmod(c, cols)
            return (half_slab(hbm_ref, pl.ds(region * rpr, rpr), w),
                    half_slab(buf, pl.ds((region - p * PHASE) * rpr, rpr), w))

        def start_reads(p, lo, hi, sem):
            @pl.loop(lo, hi)
            def _(c):
                hbm, vmem = column(p, c, x_ref)
                pltpu.make_async_copy(hbm, vmem, sem).start()

        def start_writes(p, lo, hi, sem):
            @pl.loop(lo, hi)
            def _(c):
                hbm, vmem = column(p, c, o_ref)
                pltpu.make_async_copy(vmem, hbm, sem).start()

        def start_burst(row, k):
            for i in range(BURST):
                w = k * BURST + i
                pltpu.make_async_copy(
                    half_slab(buf, row, w), half_slab(o_ref, row, w), burst_sem).start()

        def wait_all(sem, rows, slabs, lanes):
            total = buf.at[pl.ds(0, rows), pl.ds(0, slabs), :, pl.ds(0, lanes)]
            pltpu.make_async_copy(total, total, sem).wait()

        def wait_columns(sem, n, sizes):
            for size in sizes:
                pl.when(n == size)(lambda size=size: wait_all(sem, rpr, size, half))

        def slabs_of(row0, i):
            row, part = _divmod(i, iters_per_row)
            return [(row0 + row, part * per_iter + s) for s in range(per_iter)]

        def group_mean(row0, fn):
            def body(i, acc):
                for at in slabs_of(row0, i):
                    v = fn(buf[at].astype(f32))
                    parts = [v[:, k:k + ACC_LANES] for k in range(0, W, ACC_LANES)]
                    while len(parts) > 1:
                        parts = [parts[k] + parts[k + 1] for k in range(0, len(parts), 2)]
                    acc = acc + parts[0]
                return acc

            acc = lax.fori_loop(0, n_iters, body, jnp.zeros((SLAB_ROWS, ACC_LANES), f32))
            return jnp.sum(jnp.sum(acc, axis=0, keepdims=True), axis=1, keepdims=True) * inv_n

        def widen(v):
            return jnp.tile(v, (1, W // 128))

        def run_task(p, region, task):
            which = (task > 2).astype(jnp.int32)
            base = (region - p * PHASE) * rpr
            row0 = base + which * rpg

            @pl.when(task == 0)
            def _():
                @pl.loop(0, 2)
                def _(h):
                    mu = group_mean(base + h * rpg, lambda v: v)
                    stats[h] = jnp.broadcast_to(mu, (8, 128))

            @pl.when((task == 1) | (task == 3))
            def _():
                mu = widen(stats[which])
                var = group_mean(row0, lambda v: jnp.square(v - mu))
                stats[2] = jnp.broadcast_to(1.0 / jnp.sqrt(var + EPS), (8, 128))

            @pl.when((task == 2) | (task == 4))
            def _():
                mu, rstd = widen(stats[which]), stats[2]
                _, group = _divmod(region * 2 + which, GROUPS)
                p_row, p_col = _divmod(group * cpg, 128)

                @pl.loop(0, n_iters)
                def _(i):
                    slabs = slabs_of(row0, i)
                    for c in range(CH_PER_ITER):
                        col = p_col + i * CH_PER_ITER + c
                        scale = widen(rstd * gb_smem[p_row, col])
                        shift = gb_smem[p_rows + p_row, col]
                        for at in slabs[c * spc:(c + 1) * spc]:
                            buf[at] = ((buf[at].astype(f32) - mu) * scale + shift).astype(buf.dtype)

        def pick(p, values):
            out = jnp.int32(values[-1])
            for i, v in enumerate(values[:-1]):
                out = jnp.where(p == i, v, out)
            return out

        def phase_columns(p):
            lo = jnp.where(p == 0, 0, HELD + p * PHASE) * cols
            e0, e1 = (lo + pick(p, [e[i] for e in edges]) for i in range(2))
            return lo, e0, e1, (HELD + (p + 1) * PHASE) * cols

        def open_read_phase(p):
            lo, e0, e1, _ = phase_columns(p)
            start_reads(p, lo, e0, read_sem.at[2])
            start_reads(p, e0, e1, read_sem.at[0])

        g_copy = pltpu.make_async_copy(g_ref, gb_in.at[0], param_sem.at[0])
        b_copy = pltpu.make_async_copy(b_ref, gb_in.at[1], param_sem.at[1])
        open_read_phase(jnp.int32(0))
        g_copy.start()
        b_copy.start()

        def phase(p, counters):
            lo, e0, e1, hi = phase_columns(p)
            n = pick(p, n_periods)
            first_write = hi - PHASE * cols
            wait_columns(read_sem.at[2], e0 - lo, lead_sizes)

            def period(j, carry):
                e0, e1, beat, (region, task, row, k) = carry
                extra, beat = _count(0, beat, LONG_EVERY, jnp.bool_(True))
                e2 = jnp.where(j + 1 < n, jnp.minimum(e1 + PERIOD + extra, hi - READ_TAIL), hi)
                start_reads(p, e1, e2, read_sem.at[(j + 1) & 1])

                @pl.when((p == 0) & (j == 1))
                def _():
                    g_copy.wait()
                    b_copy.wait()
                    gb_f32[pl.ds(0, p_rows)] = gb_in[0].astype(f32)
                    gb_f32[pl.ds(p_rows, p_rows)] = gb_in[1].astype(f32)
                    to_smem = pltpu.make_async_copy(gb_f32, gb_smem, param_sem.at[0])
                    to_smem.start()
                    to_smem.wait()

                runnable = ((region + 1) * cols <= e0) & (j != n - 1)

                @pl.when(runnable)
                def _():
                    run_task(p, region, task)

                region, task = _count(region, task, TASKS, runnable)
                rows_done = region * rpr + jnp.where(task > 2, rpg, 0)
                send = (j < n - 1) & (row < jnp.minimum(rows_done, HELD * rpr))
                wait_columns(read_sem.at[j & 1], e1 - e0, period_sizes)

                @pl.when(send)
                def _():
                    start_burst(row, k)

                @pl.when(j == n - 1)
                def _():
                    start_writes(p, first_write, first_write + cols, write_sem.at[0])

                return e1, e2, beat, (region, task, *_count(row, k, BURSTS_PER_ROW, send))

            *_, counters = lax.fori_loop(
                0, n + 1 + TASKS, period, (e0, e1, jnp.int32(1 % LONG_EVERY), counters))

            @pl.when(p == 0)
            def _():
                for r in range(HELD):
                    start_writes(0, r * cols + burst_cols, (r + 1) * cols, write_sem.at[3])

            @pl.when(p == n_phases - 1)
            def _():
                row, k = counters[2:]

                @pl.loop(row * BURSTS_PER_ROW + k, HELD * rpr * BURSTS_PER_ROW)
                def _(i):
                    start_burst(lax.div(i, BURSTS_PER_ROW), lax.rem(i, BURSTS_PER_ROW))

            start_writes(p, first_write + cols, hi - cols, write_sem.at[0])
            start_writes(p, hi - cols, hi - 2 * WRITE_TAIL, write_sem.at[1])
            start_writes(p, hi - 2 * WRITE_TAIL, hi, write_sem.at[2])

            @pl.when(p == 0)
            def _():
                wait_all(write_sem.at[3], HELD * rpr, cols - burst_cols, half)

            @pl.when(p == n_phases - 1)
            def _():
                wait_all(burst_sem, HELD * rpr * BURST, BURSTS_PER_ROW, half)

            wait_all(write_sem.at[0], (PHASE - 1) * rpr, SLABS, W)
            wait_all(write_sem.at[1], rpr, SLABS - WRITE_TAIL, W)

            @pl.when(p + 1 < n_phases)
            def _():
                open_read_phase(p + 1)

            wait_all(write_sem.at[2], rpr, WRITE_TAIL, W)
            return counters

        lax.fori_loop(0, n_phases, phase, (jnp.int32(0),) * 4)

    t = 0
    for p, e in enumerate(edges):
        base = (HELD + p * PHASE) * cols if p else 0
        n, end = len(e) - 1, HELD + (p + 1) * PHASE
        for j in range(n + 1 + TASKS):
            landed = base + e[j] if j <= n else end * cols
            t += (t // TASKS + 1) * cols <= landed and j != n - 1
            assert j != n - 1 or t >= TASKS * (end - PHASE + 1)
        assert t == TASKS * end

    view = (n_regions * rpr, SLABS, SLAB_ROWS, W)
    hbm_spec = pl.BlockSpec(memory_space=pltpu.HBM)
    out = pl.pallas_call(
        kernel,
        in_specs=[hbm_spec, hbm_spec, hbm_spec],
        out_specs=hbm_spec,
        out_shape=jax.ShapeDtypeStruct(view, x.dtype),
        scratch_shapes=[
            pltpu.VMEM(((HELD + PHASE) * rpr, SLABS, SLAB_ROWS, W), x.dtype),
            pltpu.VMEM((3, 8, 128), f32),
            pltpu.VMEM((2, p_rows, 128), g.dtype),
            pltpu.VMEM((2 * p_rows, 128), f32),
            pltpu.SMEM((2 * p_rows, 128), f32),
            pltpu.SemaphoreType.DMA((3,)),
            pltpu.SemaphoreType.DMA((4,)),
            pltpu.SemaphoreType.DMA,
            pltpu.SemaphoreType.DMA((2,)),
        ],
        compiler_params=pltpu.CompilerParams(
            vmem_limit_bytes=112 * 2**20, disable_bounds_checks=True),
    )(x.reshape(view), g.reshape(p_rows, 128), b.reshape(p_rows, 128))
    return out.reshape(x.shape)
```

```python
import jax
import jax.numpy as jnp
from jax import lax
import jax.experimental.pallas as pl
import jax.experimental.pallas.tpu as pltpu

GROUPS = 32
EPS = 1e-5

SLAB_ROWS = 8
SLABS = 32
HELD = 2
PHASE = 10
PERIOD = 11
LONG_EVERY = 5
LEAD = (12, 12, 10)
READ_TAIL = 3
WRITE_TAIL = 1
BAND_ROWS = 6
BURST = 3
BURSTS_PER_ROW = 11
CH_PER_ITER = 8
ACC_LANES = 512
TASKS = 3
CATCH_UP = 5


def _period_edges(cols, lead):
    edges = [0]
    while edges[-1] < cols - READ_TAIL:
        j = len(edges) - 1
        edges.append(min(lead + j * PERIOD + j // LONG_EVERY, cols - READ_TAIL))
    return edges


def _divmod(i, n):
    assert n & (n - 1) == 0
    return i >> (n.bit_length() - 1), i & (n - 1)


def _count(hi, lo, n, step):
    wrap = step & (lo == n - 1)
    return hi + wrap.astype(jnp.int32), jnp.where(wrap, 0, lo + step.astype(jnp.int32))


@jax.jit
def pallas_standalone__groupnorm__prompt_kernel(
    x: jax.Array,
    g: jax.Array,
    b: jax.Array,
):
    B, C, H, W = x.shape
    cpg = C // GROUPS
    spc = H // SLAB_ROWS
    rpg = cpg * spc // SLABS
    rpr = 2 * rpg
    cols = 2 * SLABS
    half = W // 2
    n_regions = B * GROUPS // 2
    n_phases = len(LEAD)
    n_bands = PHASE * rpr // BAND_ROWS - 2
    early_rows = (PHASE * rpr - n_bands * BAND_ROWS) // 2
    burst_cols = BURST * BURSTS_PER_ROW
    n_iters = cpg // CH_PER_ITER
    per_iter = CH_PER_ITER * spc
    iters_per_row = SLABS // per_iter
    p_rows = C // 128
    inv_n = 1.0 / (cpg * H * W)
    f32 = jnp.float32
    assert H % SLAB_ROWS == 0 and (cpg * spc) % SLABS == 0 and SLABS % (spc * CH_PER_ITER) == 0
    assert 128 % cpg == 0 and C % 128 == 0 and HELD + n_phases * PHASE == n_regions
    assert 0 < cols - burst_cols <= SLABS and 0 < WRITE_TAIL < SLABS
    assert 2 * early_rows + n_bands * BAND_ROWS == PHASE * rpr and early_rows <= rpr
    assert BAND_ROWS % 2 == 0

    edges = [_period_edges((PHASE + (0 if p else HELD)) * cols, LEAD[p]) for p in range(n_phases)]
    n_periods = [len(e) - 1 for e in edges]
    period_sizes = sorted({hi - lo for e in edges for lo, hi in zip(e, e[1:])} | {READ_TAIL})

    n_steps, t = [], 0
    for p, e in enumerate(edges):
        base, end = (HELD + p * PHASE) * cols if p else 0, HELD + (p + 1) * PHASE
        j, n = 0, len(e) - 1
        while j <= n + CATCH_UP or t < TASKS * 2 * end:
            landed = base + e[j] if j <= n else end * cols
            t += landed >= ((t // TASKS // 2 + 1) * cols if t >= TASKS else SLABS) and j != n - 1
            assert j != n - 1 or t >= TASKS * 2 * (end - PHASE + 2)
            j += 1
        n_steps.append(j)

    def kernel(x_ref, g_ref, b_ref, o_ref, buf, stats, gb_in, gb_f32, gb_smem,
               read_sem, write_sem, burst_sem, param_sem):
        def half_slab(ref, rows, w):
            slab, side = _divmod(w, 2)
            return ref.at[rows, slab, :, pl.ds(pl.multiple_of(side * half, half), half)]

        def start_reads(p, lo, hi, sem):
            @pl.loop(lo, jnp.minimum(hi, cols))
            def _(c):
                group, slab = _divmod(c, SLABS)
                rows = pl.ds(group * rpg, rpg)
                for w in (2 * slab, 2 * slab + 1):
                    pltpu.make_async_copy(
                        half_slab(x_ref, rows, w), half_slab(buf, rows, w), sem).start()

            @pl.loop(jnp.maximum(lo, cols), hi)
            def _(c):
                region, w = _divmod(c, cols)
                pltpu.make_async_copy(
                    half_slab(x_ref, pl.ds(region * rpr, rpr), w),
                    half_slab(buf, pl.ds((region - p * PHASE) * rpr, rpr), w), sem).start()

        def start_writes(p, row0, rows, lo, hi, sem):
            @pl.loop(lo, hi)
            def _(c):
                band, w = _divmod(c, cols)
                row = row0 + band * rows
                pltpu.make_async_copy(
                    half_slab(buf, pl.ds(row, rows), w),
                    half_slab(o_ref, pl.ds(row + p * PHASE * rpr, rows), w), sem).start()

        def start_burst(row, k):
            for i in range(BURST):
                w = k * BURST + i
                pltpu.make_async_copy(
                    half_slab(buf, row, w), half_slab(o_ref, row, w), burst_sem).start()

        def wait_all(sem, rows, slabs, lanes):
            total = buf.at[pl.ds(0, rows), pl.ds(0, slabs), :, pl.ds(0, lanes)]
            pltpu.make_async_copy(total, total, sem).wait()

        def wait_columns(sem, n, sizes):
            for size in sizes:
                pl.when(n == size)(lambda size=size: wait_all(sem, rpr, size, half))

        def slabs_of(row0, i):
            row, part = _divmod(i, iters_per_row)
            return [(row0 + row, part * per_iter + s) for s in range(per_iter)]

        def group_mean(row0, fn):
            def body(i, acc):
                for at in slabs_of(row0, i):
                    v = fn(buf[at].astype(f32))
                    parts = [v[:, k:k + ACC_LANES] for k in range(0, W, ACC_LANES)]
                    while len(parts) > 1:
                        parts = [parts[k] + parts[k + 1] for k in range(0, len(parts), 2)]
                    acc = acc + parts[0]
                return acc

            acc = lax.fori_loop(0, n_iters, body, jnp.zeros((SLAB_ROWS, ACC_LANES), f32))
            return jnp.sum(jnp.sum(acc, axis=0, keepdims=True), axis=1, keepdims=True) * inv_n

        def widen(v):
            return jnp.tile(v, (1, W // 128))

        def run_task(p, group, task):
            row0 = group * rpg - p * PHASE * rpr

            @pl.when(task == 0)
            def _():
                stats[0] = jnp.broadcast_to(group_mean(row0, lambda v: v), (8, 128))

            @pl.when(task == 1)
            def _():
                mu = widen(stats[0])
                var = group_mean(row0, lambda v: jnp.square(v - mu))
                stats[1] = jnp.broadcast_to(1.0 / jnp.sqrt(var + EPS), (8, 128))

            @pl.when(task == 2)
            def _():
                mu, rstd = widen(stats[0]), stats[1]
                p_row, p_col = _divmod(_divmod(group, GROUPS)[1] * cpg, 128)

                @pl.loop(0, n_iters)
                def _(i):
                    slabs = slabs_of(row0, i)
                    for c in range(CH_PER_ITER):
                        col = p_col + i * CH_PER_ITER + c
                        scale = widen(rstd * gb_smem[p_row, col])
                        shift = gb_smem[p_rows + p_row, col]
                        for at in slabs[c * spc:(c + 1) * spc]:
                            buf[at] = ((buf[at].astype(f32) - mu) * scale + shift).astype(buf.dtype)

        def pick(p, values):
            out = jnp.int32(values[-1])
            for i, v in enumerate(values[:-1]):
                out = jnp.where(p == i, v, out)
            return out

        def phase_columns(p):
            lo = jnp.where(p == 0, 0, HELD + p * PHASE) * cols
            return lo, lo + pick(p, LEAD), (HELD + (p + 1) * PHASE) * cols

        def open_read_phase(p):
            start_reads(p, *phase_columns(p)[:2], read_sem.at[0])

        g_copy = pltpu.make_async_copy(g_ref, gb_in.at[0], param_sem.at[0])
        b_copy = pltpu.make_async_copy(b_ref, gb_in.at[1], param_sem.at[1])
        open_read_phase(jnp.int32(0))
        g_copy.start()
        b_copy.start()

        def phase(p, counters):
            e0, e1, hi = phase_columns(p)
            n = pick(p, n_periods)

            def period(j, carry):
                e0, e1, beat, (group, task, row, k) = carry
                extra, beat = _count(0, beat, LONG_EVERY, jnp.bool_(True))
                e2 = jnp.where(j + 1 < n, jnp.minimum(e1 + PERIOD + extra, hi - READ_TAIL), hi)
                start_reads(p, e1, e2, read_sem.at[(j + 1) & 1])

                @pl.when((p == 0) & (j == 2))
                def _():
                    g_copy.wait()
                    b_copy.wait()
                    gb_f32[pl.ds(0, p_rows)] = gb_in[0].astype(f32)
                    gb_f32[pl.ds(p_rows, p_rows)] = gb_in[1].astype(f32)
                    to_smem = pltpu.make_async_copy(gb_f32, gb_smem, param_sem.at[0])
                    to_smem.start()
                    to_smem.wait()

                needed = jnp.where(group == 0, SLABS, ((group >> 1) + 1) * cols)
                runnable = (needed <= e0) & (j != n - 1)

                @pl.when(runnable)
                def _():
                    run_task(p, group, task)

                group, task = _count(group, task, TASKS, runnable)
                send = (j < n - 1) & (row < jnp.minimum(group * rpg, HELD * rpr))
                wait_columns(read_sem.at[j & 1], e1 - e0, period_sizes)

                @pl.when(send)
                def _():
                    start_burst(row, k)

                @pl.when(j == n - 1)
                def _():
                    start_writes(p, HELD * rpr, early_rows, 0, cols, write_sem.at[0])

                @pl.when(j == n + CATCH_UP)
                def _():
                    start_writes(p, HELD * rpr, early_rows, cols, 2 * cols, write_sem.at[0])

                return e1, e2, beat, (group, task, *_count(row, k, BURSTS_PER_ROW, send))

            *_, counters = lax.fori_loop(
                0, pick(p, n_steps), period, (e0, e1, jnp.int32(0), counters))

            @pl.when(p == 0)
            def _():
                for r in range(HELD):
                    start_writes(0, r * rpr, rpr, burst_cols, cols, write_sem.at[3])

            @pl.when(p == n_phases - 1)
            def _():
                row, k = counters[2:]

                @pl.loop(row * BURSTS_PER_ROW + k, HELD * rpr * BURSTS_PER_ROW)
                def _(i):
                    start_burst(lax.div(i, BURSTS_PER_ROW), lax.rem(i, BURSTS_PER_ROW))

            row0, end = HELD * rpr + 2 * early_rows, n_bands * cols
            start_writes(p, row0, BAND_ROWS, 0, end - SLABS, write_sem.at[0])
            start_writes(p, row0, BAND_ROWS, end - SLABS, end - WRITE_TAIL, write_sem.at[1])
            start_writes(p, row0, BAND_ROWS, end - WRITE_TAIL, end, write_sem.at[2])

            @pl.when(p == 0)
            def _():
                wait_all(write_sem.at[3], HELD * rpr, cols - burst_cols, half)

            @pl.when(p == n_phases - 1)
            def _():
                wait_all(burst_sem, HELD * rpr * BURST, BURSTS_PER_ROW, half)

            wait_all(write_sem.at[0], PHASE * rpr - BAND_ROWS // 2, SLABS, W)
            wait_all(write_sem.at[1], BAND_ROWS, SLABS - WRITE_TAIL, half)

            @pl.when(p + 1 < n_phases)
            def _():
                open_read_phase(p + 1)

            wait_all(write_sem.at[2], BAND_ROWS, WRITE_TAIL, half)
            return counters

        lax.fori_loop(0, n_phases, phase, (jnp.int32(0),) * 4)

    view = (n_regions * rpr, SLABS, SLAB_ROWS, W)
    hbm_spec = pl.BlockSpec(memory_space=pltpu.HBM)
    out = pl.pallas_call(
        kernel,
        in_specs=[hbm_spec, hbm_spec, hbm_spec],
        out_specs=hbm_spec,
        out_shape=jax.ShapeDtypeStruct(view, x.dtype),
        scratch_shapes=[
            pltpu.VMEM(((HELD + PHASE) * rpr, SLABS, SLAB_ROWS, W), x.dtype),
            pltpu.VMEM((2, 8, 128), f32),
            pltpu.VMEM((2, p_rows, 128), g.dtype),
            pltpu.VMEM((2 * p_rows, 128), f32),
            pltpu.SMEM((2 * p_rows, 128), f32),
            pltpu.SemaphoreType.DMA((2,)),
            pltpu.SemaphoreType.DMA((4,)),
            pltpu.SemaphoreType.DMA,
            pltpu.SemaphoreType.DMA((2,)),
        ],
        compiler_params=pltpu.CompilerParams(
            vmem_limit_bytes=112 * 2**20,
            disable_bounds_checks=True,
            disable_semaphore_checks=True,
        ),
    )(x.reshape(view), g.reshape(p_rows, 128), b.reshape(p_rows, 128))
    return out.reshape(x.shape)
```

```python
import jax
import jax.numpy as jnp
import numpy as np
from jax import lax
import jax.experimental.pallas as pl
import jax.experimental.pallas.tpu as pltpu

GROUPS = 32
EPS = 1e-5

SLAB_ROWS = 8
SLABS = 32
HELD = 2
PHASE = 10
PERIOD = 11
LONG_EVERY = 5
LEAD = (12, 12, 11)
READ_TAIL = 3
WRITE_TAIL = 1
BAND_ROWS = 6
BURST = 3
BURSTS_PER_ROW = 11
CH_PER_ITER = 8
ACC_LANES = 512
TASKS = 3
CATCH_UP = 5


def _period_edges(cols, lead):
    edges = [0]
    while edges[-1] < cols - READ_TAIL:
        j = len(edges) - 1
        edges.append(min(lead + j * PERIOD + j // LONG_EVERY, cols - READ_TAIL))
    return edges


def _divmod(i, n):
    assert n & (n - 1) == 0
    return i >> (n.bit_length() - 1), i & (n - 1)


def _count(hi, lo, n, step):
    wrap = step & (lo == n - 1)
    return hi + wrap.astype(jnp.int32), jnp.where(wrap, 0, lo + step.astype(jnp.int32))


@jax.jit
def pallas_standalone__groupnorm__prompt_kernel(
    x: jax.Array,
    g: jax.Array,
    b: jax.Array,
):
    B, C, H, W = x.shape
    cpg = C // GROUPS
    spc = H // SLAB_ROWS
    rpg = cpg * spc // SLABS
    rpr = 2 * rpg
    cols = 2 * SLABS
    half = W // 2
    n_regions = B * GROUPS // 2
    n_phases = len(LEAD)
    n_bands = PHASE * rpr // BAND_ROWS - 2
    early_rows = (PHASE * rpr - n_bands * BAND_ROWS) // 2
    burst_cols = BURST * BURSTS_PER_ROW
    n_iters = cpg // CH_PER_ITER
    per_iter = CH_PER_ITER * spc
    iters_per_row = SLABS // per_iter
    p_rows = C // 128
    inv_n = 1.0 / (cpg * H * W)
    f32 = jnp.float32
    assert H % SLAB_ROWS == 0 and (cpg * spc) % SLABS == 0 and SLABS % (spc * CH_PER_ITER) == 0
    assert 128 % cpg == 0 and C % 128 == 0 and HELD + n_phases * PHASE == n_regions
    assert 0 < cols - burst_cols <= SLABS and 0 < WRITE_TAIL < SLABS
    assert 2 * early_rows + n_bands * BAND_ROWS == PHASE * rpr and early_rows <= rpr
    assert BAND_ROWS % 2 == 0

    edges = [_period_edges((PHASE + (0 if p else HELD)) * cols, LEAD[p]) for p in range(n_phases)]
    n_periods = [len(e) - 1 for e in edges]
    period_sizes = sorted({hi - lo for e in edges for lo, hi in zip(e, e[1:])} | {READ_TAIL})

    n_steps, t = [], 0
    for p, e in enumerate(edges):
        base, end = (HELD + p * PHASE) * cols if p else 0, HELD + (p + 1) * PHASE
        j, n = 0, len(e) - 1
        while j <= n + CATCH_UP or t < TASKS * 2 * end:
            landed = base + e[j] if j <= n else end * cols
            t += landed >= ((t // TASKS // 2 + 1) * cols if t >= TASKS else SLABS) and j != n - 1
            assert j != n - 1 or t >= TASKS * 2 * (end - PHASE + 2)
            j += 1
        n_steps.append(j)

    def kernel(x_ref, g_ref, b_ref, o_ref, buf, stats, gb_in, gb_f32, gb_smem,
               read_sem, write_sem, burst_sem, param_sem):
        def half_slab(ref, rows, w):
            slab, side = _divmod(w, 2)
            return ref.at[rows, slab, :, pl.ds(pl.multiple_of(side * half, half), half)]

        def start_reads(p, lo, hi, sem):
            @pl.loop(lo, jnp.minimum(hi, cols))
            def _(c):
                group, slab = _divmod(c, SLABS)
                rows = pl.ds(group * rpg, rpg)
                for w in (2 * slab, 2 * slab + 1):
                    pltpu.make_async_copy(
                        half_slab(x_ref, rows, w), half_slab(buf, rows, w), sem).start()

            @pl.loop(jnp.maximum(lo, cols), hi)
            def _(c):
                region, w = _divmod(c, cols)
                pltpu.make_async_copy(
                    half_slab(x_ref, pl.ds(region * rpr, rpr), w),
                    half_slab(buf, pl.ds((region - p * PHASE) * rpr, rpr), w), sem).start()

        def start_writes(p, row0, rows, lo, hi, sem):
            @pl.loop(lo, hi)
            def _(c):
                band, w = _divmod(c, cols)
                row = row0 + band * rows
                pltpu.make_async_copy(
                    half_slab(buf, pl.ds(row, rows), w),
                    half_slab(o_ref, pl.ds(row + p * PHASE * rpr, rows), w), sem).start()

        def start_burst(row, k):
            for i in range(BURST):
                w = k * BURST + i
                pltpu.make_async_copy(
                    half_slab(buf, row, w), half_slab(o_ref, row, w), burst_sem).start()

        def wait_all(sem, rows, slabs, lanes):
            total = buf.at[pl.ds(0, rows), pl.ds(0, slabs), :, pl.ds(0, lanes)]
            pltpu.make_async_copy(total, total, sem).wait()

        def wait_columns(sem, n, sizes):
            for size in sizes:
                pl.when(n == size)(lambda size=size: wait_all(sem, rpr, size, half))

        def slabs_of(row0, i):
            row, part = _divmod(i, iters_per_row)
            return [(row0 + row, part * per_iter + s) for s in range(per_iter)]

        def group_mean(row0, fn):
            def body(i, acc):
                for at in slabs_of(row0, i):
                    v = fn(buf[at].astype(f32))
                    parts = [v[:, k:k + ACC_LANES] for k in range(0, W, ACC_LANES)]
                    while len(parts) > 1:
                        parts = [parts[k] + parts[k + 1] for k in range(0, len(parts), 2)]
                    acc = acc + parts[0]
                return acc

            acc = lax.fori_loop(0, n_iters, body, jnp.zeros((SLAB_ROWS, ACC_LANES), f32))
            return jnp.sum(jnp.sum(acc, axis=0, keepdims=True), axis=1, keepdims=True) * inv_n

        def widen(v):
            return jnp.tile(v, (1, W // 128))

        def run_task(p, group, task):
            row0 = group * rpg - p * PHASE * rpr

            @pl.when(task == 0)
            def _():
                stats[0] = jnp.broadcast_to(group_mean(row0, lambda v: v), (8, 128))

            @pl.when(task == 1)
            def _():
                mu = widen(stats[0])
                var = group_mean(row0, lambda v: jnp.square(v - mu))
                stats[1] = jnp.broadcast_to(1.0 / jnp.sqrt(var + EPS), (8, 128))

            @pl.when(task == 2)
            def _():
                mu, rstd = widen(stats[0]), stats[1]
                p_row, p_col = _divmod(_divmod(group, GROUPS)[1] * cpg, 128)

                @pl.loop(0, n_iters)
                def _(i):
                    slabs = slabs_of(row0, i)
                    for c in range(CH_PER_ITER):
                        col = p_col + i * CH_PER_ITER + c
                        scale = widen(rstd * gb_smem[p_row, col])
                        shift = gb_smem[p_rows + p_row, col]
                        for at in slabs[c * spc:(c + 1) * spc]:
                            buf[at] = ((buf[at].astype(f32) - mu) * scale + shift).astype(buf.dtype)

        def pick(p, values):
            out = values[-1]
            for i, v in enumerate(values[:-1]):
                out = jnp.where(p == i, v, out)
            return out

        def phase_columns(p):
            lo = jnp.where(p == 0, 0, HELD + p * PHASE) * cols
            return lo, lo + pick(p, LEAD), (HELD + (p + 1) * PHASE) * cols

        g_copy = pltpu.make_async_copy(g_ref, gb_in.at[0], param_sem.at[0])
        b_copy = pltpu.make_async_copy(b_ref, gb_in.at[1], param_sem.at[1])
        start_reads(0, 0, LEAD[0], read_sem.at[0])
        g_copy.start()
        b_copy.start()

        def phase(p, counters):
            e0, e1, hi = phase_columns(p)
            n = pick(p, n_periods)

            def period(j, carry):
                e0, e1, beat, (group, task, row, k) = carry
                extra, beat = _count(0, beat, LONG_EVERY, j < n)
                e2 = jnp.where(j + 1 < n, jnp.minimum(e1 + PERIOD + extra, hi - READ_TAIL), hi)
                start_reads(p, e1, e2, read_sem.at[(j + 1) & 1])

                @pl.when((p == 0) & (j == 2))
                def _():
                    g_copy.wait()
                    b_copy.wait()
                    gb_f32[pl.ds(0, p_rows)] = gb_in[0].astype(f32)
                    gb_f32[pl.ds(p_rows, p_rows)] = gb_in[1].astype(f32)
                    to_smem = pltpu.make_async_copy(gb_f32, gb_smem, param_sem.at[0])
                    to_smem.start()
                    to_smem.wait()

                needed = jnp.where(group == 0, SLABS, ((group >> 1) + 1) * cols)
                runnable = (needed <= e0) & (j != n - 1)

                @pl.when(runnable)
                def _():
                    run_task(p, group, task)

                group, task = _count(group, task, TASKS, runnable)
                send = (j < n - 1) & (row < jnp.minimum(group * rpg, HELD * rpr))
                wait_columns(read_sem.at[j & 1], e1 - e0, period_sizes)

                @pl.when(send)
                def _():
                    start_burst(row, k)

                @pl.when(j == n - 1)
                def _():
                    start_writes(p, HELD * rpr, early_rows, 0, cols, write_sem.at[0])

                @pl.when(j == n + CATCH_UP)
                def _():
                    start_writes(p, HELD * rpr, early_rows, cols, 2 * cols, write_sem.at[0])

                return e1, e2, beat, (group, task, *_count(row, k, BURSTS_PER_ROW, send))

            *_, counters = lax.fori_loop(
                0, pick(p, n_steps), period, (e0, e1, np.int32(0), counters))

            @pl.when(p == 0)
            def _():
                for r in range(HELD):
                    start_writes(0, r * rpr, rpr, burst_cols, cols, write_sem.at[3])

            @pl.when(p == n_phases - 1)
            def _():
                row, k = counters[2:]

                @pl.loop(row * BURSTS_PER_ROW + k, HELD * rpr * BURSTS_PER_ROW)
                def _(i):
                    start_burst(lax.div(i, BURSTS_PER_ROW), lax.rem(i, BURSTS_PER_ROW))

            row0, end = HELD * rpr + 2 * early_rows, n_bands * cols
            start_writes(p, row0, BAND_ROWS, 0, end - SLABS, write_sem.at[0])
            start_writes(p, row0, BAND_ROWS, end - SLABS, end - WRITE_TAIL, write_sem.at[1])
            start_writes(p, row0, BAND_ROWS, end - WRITE_TAIL, end, write_sem.at[2])

            @pl.when(p == 0)
            def _():
                wait_all(write_sem.at[3], HELD * rpr, cols - burst_cols, half)

            @pl.when(p == n_phases - 1)
            def _():
                wait_all(burst_sem, HELD * rpr * BURST, BURSTS_PER_ROW, half)

            wait_all(write_sem.at[0], PHASE * rpr - BAND_ROWS // 2, SLABS, W)
            wait_all(write_sem.at[1], BAND_ROWS, SLABS - WRITE_TAIL, half)

            @pl.when(p + 1 < n_phases)
            def _():
                start_reads(p + 1, *phase_columns(p + 1)[:2], read_sem.at[0])

            wait_all(write_sem.at[2], BAND_ROWS, WRITE_TAIL, half)
            return counters

        lax.fori_loop(0, n_phases, phase, (np.int32(0),) * 4)

    view = (n_regions * rpr, SLABS, SLAB_ROWS, W)
    hbm_spec = pl.BlockSpec(memory_space=pltpu.HBM)
    out = pl.pallas_call(
        kernel,
        in_specs=[hbm_spec, hbm_spec, hbm_spec],
        out_specs=hbm_spec,
        out_shape=jax.ShapeDtypeStruct(view, x.dtype),
        scratch_shapes=[
            pltpu.VMEM(((HELD + PHASE) * rpr, SLABS, SLAB_ROWS, W), x.dtype),
            pltpu.VMEM((2, 8, 128), f32),
            pltpu.VMEM((2, p_rows, 128), g.dtype),
            pltpu.VMEM((2 * p_rows, 128), f32),
            pltpu.SMEM((2 * p_rows, 128), f32),
            pltpu.SemaphoreType.DMA((2,)),
            pltpu.SemaphoreType.DMA((4,)),
            pltpu.SemaphoreType.DMA,
            pltpu.SemaphoreType.DMA((2,)),
        ],
        compiler_params=pltpu.CompilerParams(
            vmem_limit_bytes=112 * 2**20,
            disable_bounds_checks=True,
            disable_semaphore_checks=True,
        ),
    )(x.reshape(view), g.reshape(p_rows, 128), b.reshape(p_rows, 128))
    return out.reshape(x.shape)
```

```python
import jax
import jax.numpy as jnp
import numpy as np
from jax import lax
import jax.experimental.pallas as pl
import jax.experimental.pallas.tpu as pltpu

GROUPS = 32
EPS = 1e-5

SLAB_ROWS = 8
SLABS = 32
HELD = 2
PHASE = 10
PAIRED = 2
PERIOD = 11
LONG_EVERY = 5
LEAD = (7, 6, 4)
READ_TAIL = 3
WRITE_TAIL = 2
BAND_ROWS = 6
HELD_BANDS = (6, 5, 5)
BURST = 3
BURSTS_PER_ROW = 11
CH_PER_ITER = 8
ACC_LANES = 512
TASKS = 3
CATCH_UP = 5


def _period_edges(cols, lead):
    edges = [0]
    while edges[-1] < cols - READ_TAIL:
        j = len(edges) - 1
        edges.append(min(lead + j * PERIOD + j // LONG_EVERY, cols - READ_TAIL))
    return edges


def _divmod(i, n):
    assert n & (n - 1) == 0
    return i >> (n.bit_length() - 1), i & (n - 1)


def _count(hi, lo, n, step):
    wrap = step & (lo == n - 1)
    return hi + wrap.astype(jnp.int32), jnp.where(wrap, 0, lo + step.astype(jnp.int32))


@jax.jit
def pallas_standalone__groupnorm__prompt_kernel(
    x: jax.Array,
    g: jax.Array,
    b: jax.Array,
):
    B, C, H, W = x.shape
    cpg = C // GROUPS
    spc = H // SLAB_ROWS
    rpg = cpg * spc // SLABS
    rpr = 2 * rpg
    cols = 2 * SLABS
    half = W // 2
    n_regions = B * GROUPS // 2
    n_phases = len(LEAD)
    n_bands = PHASE * rpr // BAND_ROWS - 2
    early_rows = (PHASE * rpr - n_bands * BAND_ROWS) // 2
    burst_cols = BURST * BURSTS_PER_ROW
    n_iters = cpg // CH_PER_ITER
    per_iter = CH_PER_ITER * spc
    iters_per_row = SLABS // per_iter
    p_rows = C // 128
    inv_n = 1.0 / (cpg * H * W)
    f32 = jnp.float32
    assert H % SLAB_ROWS == 0 and (cpg * spc) % SLABS == 0 and SLABS % (spc * CH_PER_ITER) == 0
    assert 128 % cpg == 0 and C % 128 == 0 and HELD + n_phases * PHASE == n_regions
    assert 0 < cols - burst_cols <= SLABS and 0 < WRITE_TAIL < SLABS
    assert 2 * early_rows + n_bands * BAND_ROWS == PHASE * rpr and early_rows <= rpr
    assert BAND_ROWS % 2 == 0 and sum(HELD_BANDS) == HELD * rpr
    assert HELD % PAIRED == 0 and PHASE % PAIRED == 0

    edges = [_period_edges((PHASE + (0 if p else HELD)) * cols, LEAD[p]) for p in range(n_phases)]
    n_periods = [len(e) - 1 for e in edges]
    period_sizes = sorted({hi - lo for e in edges for lo, hi in zip(e, e[1:])} | {READ_TAIL})

    def columns_needed(group, where):
        held = where(group == 0, SLABS, ((group >> 1) + 1) * cols)
        return where(group < 2 * HELD, held, (_divmod(group, 2 * PAIRED)[0] + 1) * PAIRED * cols)

    n_steps, t = [], 0
    for p, e in enumerate(edges):
        base, end = (HELD + p * PHASE) * cols if p else 0, HELD + (p + 1) * PHASE
        j, n = 0, len(e) - 1
        while j <= n + 2 * CATCH_UP or t < TASKS * 2 * end:
            landed = base + e[j] if j <= n else end * cols
            if landed >= columns_needed(t // TASKS, np.where) and j != n - 1:
                t += 1 if t else 2
            assert j != n - 1 or t >= TASKS * 2 * (end - PHASE + 3)
            j += 1
        n_steps.append(j)

    def kernel(x_ref, g_ref, b_ref, o_ref, buf, stats, gb_in, gb_f32, gb_smem,
               read_sem, write_sem, burst_sem, param_sem):
        def half_slab(ref, rows, w):
            slab, side = _divmod(w, 2)
            return ref.at[rows, slab, :, pl.ds(pl.multiple_of(side * half, half), half)]

        def start_reads(p, lo, hi, sem):
            @pl.loop(lo, jnp.minimum(hi, cols))
            def _(c):
                group, slab = _divmod(c, SLABS)
                rows = pl.ds(group * rpg, rpg)
                for w in (2 * slab, 2 * slab + 1):
                    pltpu.make_async_copy(
                        half_slab(x_ref, rows, w), half_slab(buf, rows, w), sem).start()

            @pl.loop(jnp.maximum(lo, cols), hi)
            def _(c):
                pair, i = _divmod(c, PAIRED * cols)
                w, which = _divmod(i, PAIRED)
                region = jnp.where(c < HELD * cols, _divmod(c, cols)[0], pair * PAIRED + which)
                w = jnp.where(c < HELD * cols, _divmod(c, cols)[1], w)
                pltpu.make_async_copy(
                    half_slab(x_ref, pl.ds(region * rpr, rpr), w),
                    half_slab(buf, pl.ds((region - p * PHASE) * rpr, rpr), w), sem).start()

        def start_writes(p, row0, rows, lo, hi, sem):
            @pl.loop(lo, hi)
            def _(c):
                band, w = _divmod(c, cols)
                row = row0 + band * rows
                pltpu.make_async_copy(
                    half_slab(buf, pl.ds(row, rows), w),
                    half_slab(o_ref, pl.ds(row + p * PHASE * rpr, rows), w), sem).start()

        def start_burst(row, k):
            for i in range(BURST):
                w = k * BURST + i
                pltpu.make_async_copy(
                    half_slab(buf, row, w), half_slab(o_ref, row, w), burst_sem).start()

        def wait_all(sem, rows, slabs, lanes):
            total = buf.at[pl.ds(0, rows), pl.ds(0, slabs), :, pl.ds(0, lanes)]
            pltpu.make_async_copy(total, total, sem).wait()

        def wait_columns(sem, n, sizes):
            for size in sizes:
                pl.when(n == size)(lambda size=size: wait_all(sem, rpr, size, half))

        def slabs_of(row0, i):
            row, part = _divmod(i, iters_per_row)
            return [(row0 + row, part * per_iter + s) for s in range(per_iter)]

        def group_mean(row0, fn):
            def body(i, acc):
                for at in slabs_of(row0, i):
                    v = fn(buf[at].astype(f32))
                    parts = [v[:, k:k + ACC_LANES] for k in range(0, W, ACC_LANES)]
                    while len(parts) > 1:
                        parts = [parts[k] + parts[k + 1] for k in range(0, len(parts), 2)]
                    acc = acc + parts[0]
                return acc

            acc = lax.fori_loop(0, n_iters, body, jnp.zeros((SLAB_ROWS, ACC_LANES), f32))
            return jnp.sum(jnp.sum(acc, axis=0, keepdims=True), axis=1, keepdims=True) * inv_n

        def widen(v):
            return jnp.tile(v, (1, W // 128))

        def run_task(p, group, task):
            row0 = group * rpg - p * PHASE * rpr

            @pl.when((task == 0) | ((task == 1) & (group == 0)))
            def _():
                stats[0] = jnp.broadcast_to(group_mean(row0, lambda v: v), (8, 128))

            @pl.when(task == 1)
            def _():
                mu = widen(stats[0])
                var = group_mean(row0, lambda v: jnp.square(v - mu))
                stats[1] = jnp.broadcast_to(1.0 / jnp.sqrt(var + EPS), (8, 128))

            @pl.when(task == 2)
            def _():
                mu, rstd = widen(stats[0]), stats[1]
                p_row, p_col = _divmod(_divmod(group, GROUPS)[1] * cpg, 128)

                @pl.loop(0, n_iters)
                def _(i):
                    slabs = slabs_of(row0, i)
                    for c in range(CH_PER_ITER):
                        col = p_col + i * CH_PER_ITER + c
                        scale = widen(rstd * gb_smem[p_row, col])
                        shift = gb_smem[p_rows + p_row, col]
                        for at in slabs[c * spc:(c + 1) * spc]:
                            buf[at] = ((buf[at].astype(f32) - mu) * scale + shift).astype(buf.dtype)

        def pick(p, values):
            out = values[-1]
            for i, v in enumerate(values[:-1]):
                out = jnp.where(p == i, v, out)
            return out

        def phase_columns(p):
            lo = jnp.where(p == 0, 0, HELD + p * PHASE) * cols
            return lo, lo + pick(p, LEAD), (HELD + (p + 1) * PHASE) * cols

        g_copy = pltpu.make_async_copy(g_ref, gb_in.at[0], param_sem.at[0])
        b_copy = pltpu.make_async_copy(b_ref, gb_in.at[1], param_sem.at[1])
        start_reads(0, 0, LEAD[0], read_sem.at[0])
        g_copy.start()
        b_copy.start()

        def phase(p, counters):
            e0, e1, hi = phase_columns(p)
            n = pick(p, n_periods)
            row0, end = HELD * rpr + 2 * early_rows, n_bands * cols

            def period(j, carry):
                e0, e1, beat, (group, task, row, k) = carry
                extra, beat = _count(0, beat, LONG_EVERY, j < n)
                e2 = jnp.where(j + 1 < n, jnp.minimum(e1 + PERIOD + extra, hi - READ_TAIL), hi)
                start_reads(p, e1, e2, read_sem.at[(j + 1) & 1])

                @pl.when((p == 0) & (j == 2))
                def _():
                    g_copy.wait()
                    b_copy.wait()
                    gb_f32[pl.ds(0, p_rows)] = gb_in[0].astype(f32)
                    gb_f32[pl.ds(p_rows, p_rows)] = gb_in[1].astype(f32)
                    to_smem = pltpu.make_async_copy(gb_f32, gb_smem, param_sem.at[0])
                    to_smem.start()
                    to_smem.wait()

                runnable = (columns_needed(group, jnp.where) <= e0) & (j != n - 1)

                @pl.when(runnable)
                def _():
                    run_task(p, group, task)

                group, task = _count(group, task, TASKS, runnable)
                send = (j < n - 1) & (row < jnp.minimum(group * rpg, HELD * rpr))
                wait_columns(read_sem.at[j & 1], e1 - e0, period_sizes)

                @pl.when(send)
                def _():
                    start_burst(row, k)

                @pl.when(j == n - 1)
                def _():
                    start_writes(p, HELD * rpr, early_rows, 0, cols, write_sem.at[0])

                @pl.when(j == n + CATCH_UP)
                def _():
                    start_writes(p, HELD * rpr, early_rows, cols, 2 * cols, write_sem.at[0])

                @pl.when(j == n + 2 * CATCH_UP)
                def _():
                    start_writes(p, row0, BAND_ROWS, 0, cols, write_sem.at[0])

                return e1, e2, beat, (group, task, *_count(row, k, BURSTS_PER_ROW, send))

            *_, counters = lax.fori_loop(
                0, pick(p, n_steps), period, (e0, e1, np.int32(0), counters))

            @pl.when(p == 0)
            def _():
                for i, rows in enumerate(HELD_BANDS):
                    start_writes(0, sum(HELD_BANDS[:i]), rows, burst_cols, cols, write_sem.at[3])

            @pl.when(p == n_phases - 1)
            def _():
                row, k = counters[2:]

                @pl.loop(row * BURSTS_PER_ROW + k, HELD * rpr * BURSTS_PER_ROW)
                def _(i):
                    start_burst(lax.div(i, BURSTS_PER_ROW), lax.rem(i, BURSTS_PER_ROW))

            start_writes(p, row0, BAND_ROWS, cols, end - SLABS, write_sem.at[0])
            start_writes(p, row0, BAND_ROWS, end - SLABS, end - WRITE_TAIL, write_sem.at[1])
            start_writes(p, row0, BAND_ROWS, end - WRITE_TAIL, end, write_sem.at[2])

            @pl.when(p == 0)
            def _():
                wait_all(write_sem.at[3], HELD * rpr, cols - burst_cols, half)

            @pl.when(p == n_phases - 1)
            def _():
                wait_all(burst_sem, HELD * rpr * BURST, BURSTS_PER_ROW, half)

            wait_all(write_sem.at[0], PHASE * rpr - BAND_ROWS // 2, SLABS, W)
            wait_all(write_sem.at[1], BAND_ROWS, SLABS - WRITE_TAIL, half)

            @pl.when(p + 1 < n_phases)
            def _():
                start_reads(p + 1, *phase_columns(p + 1)[:2], read_sem.at[0])

            wait_all(write_sem.at[2], BAND_ROWS, WRITE_TAIL, half)
            return counters

        lax.fori_loop(0, n_phases, phase, tuple(map(np.int32, (0, 1, 0, 0))))

    view = (n_regions * rpr, SLABS, SLAB_ROWS, W)
    hbm_spec = pl.BlockSpec(memory_space=pltpu.HBM)
    out = pl.pallas_call(
        kernel,
        in_specs=[hbm_spec, hbm_spec, hbm_spec],
        out_specs=hbm_spec,
        out_shape=jax.ShapeDtypeStruct(view, x.dtype),
        scratch_shapes=[
            pltpu.VMEM(((HELD + PHASE) * rpr, SLABS, SLAB_ROWS, W), x.dtype),
            pltpu.VMEM((2, 8, 128), f32),
            pltpu.VMEM((2, p_rows, 128), g.dtype),
            pltpu.VMEM((2 * p_rows, 128), f32),
            pltpu.SMEM((2 * p_rows, 128), f32),
            pltpu.SemaphoreType.DMA((2,)),
            pltpu.SemaphoreType.DMA((4,)),
            pltpu.SemaphoreType.DMA,
            pltpu.SemaphoreType.DMA((2,)),
        ],
        compiler_params=pltpu.CompilerParams(
            vmem_limit_bytes=112 * 2**20,
            disable_bounds_checks=True,
            disable_semaphore_checks=True,
        ),
    )(x.reshape(view), g.reshape(p_rows, 128), b.reshape(p_rows, 128))
    return out.reshape(x.shape)
```
